```python
import jax
import jax.numpy as jnp

def _softmax(x, axis=-1):
    return jax.nn.softmax(x, axis=axis)

def _gelu(x):
    return jax.nn.gelu(x, approximate=True)

def _silu(x):
    return jax.nn.silu(x)

def _sigmoid(x):
    return jax.nn.sigmoid(x)

def _layernorm(x, axis=-1, eps=1e-05):
    m = jnp.mean(x, axis=axis, keepdims=True)
    v = jnp.var(x, axis=axis, keepdims=True)
    return (x - m) / jnp.sqrt(v + eps)

def _scatter_add(tgt, idx, src, axis=0):
    return tgt.at[idx].add(src)

def _segment_sum(src, seg, n):
    return jax.ops.segment_sum(src, seg, n)

class _Rng:

    def __init__(self, key):
        self._k = key

    def _next(self):
        self._k, sub = jax.random.split(self._k)
        return sub

    def normal(self, shape):
        return jax.random.normal(self._next(), shape, dtype=jnp.bfloat16)

    def randint(self, lo, hi, shape):
        return jax.random.randint(self._next(), shape, lo, hi, dtype=jnp.int32)

    def uniform(self, shape, lo=0.0, hi=1.0):
        return jax.random.uniform(self._next(), shape, jnp.bfloat16, lo, hi)

    def permutation(self, n):
        return jax.random.permutation(self._next(), n)
kernel_name = 'adaLN_cond__compressed_kv_cla__dense_activation_relu__decode'

def setup_inputs():
    _rng = _Rng(jax.random.key(int.from_bytes(__import__("os").urandom(4), "little")))
    _w = lambda a: (lambda t: t.astype(jnp.bfloat16) if jnp.issubdtype(t.dtype, jnp.floating) else t)(jnp.asarray(a))

    def _A_setup():
        B, H, Sq, Sk, D, M = (8, 32, 1, 4096, 128, 512)
        Dc = 4 * D
        return {'x': _w((lambda *s: _rng.normal(s) * 0.05)(B, Sq, M)), 'c_kv': _w((lambda *s: _rng.normal(s) * 0.05)(B, Sk, Dc)), 'w_q': _w((lambda *s: _rng.normal(s) * 0.05)(M, H, D) * M ** (-0.5)), 'w_uk': _w((lambda *s: _rng.normal(s) * 0.05)(Dc, H, D) * Dc ** (-0.5)), 'w_uv': _w((lambda *s: _rng.normal(s) * 0.05)(Dc, H, D) * Dc ** (-0.5)), 'w_o': _w((lambda *s: _rng.normal(s) * 0.05)(H, D, M) * (H * D) ** (-0.5))}
    _A_in = _A_setup()

    def _B_setup():
        B, S, D, Dff = (8, 1, 512, 1792)
        return {'x': _w((lambda *s: _rng.normal(s) * 0.05)(B, S, D)), 'w1': _w((lambda *s: _rng.normal(s) * 0.05)(D, Dff)), 'w2': _w((lambda *s: _rng.normal(s) * 0.05)(Dff, D))}
    _B_in = _B_setup()
    return {'A_x': _A_in['x'], 'A_c_kv': _A_in['c_kv'], 'A_w_q': _A_in['w_q'], 'A_w_uk': _A_in['w_uk'], 'A_w_uv': _A_in['w_uv'], 'A_w_o': _A_in['w_o'], 'B_x': _B_in['x'], 'B_w1': _B_in['w1'], 'B_w2': _B_in['w2'], 'c': _w((lambda *s: _rng.normal(s) * 0.05)(8, 512)), 'w_mod': _w((lambda *s: _rng.normal(s) * 0.05)(512, 6 * 512) * 512 ** (-0.5))}

def reference(A_x, A_c_kv, A_w_q, A_w_uk, A_w_uv, A_w_o, B_x, B_w1, B_w2, c, w_mod):

    def _A_ref(x, c_kv, w_q, w_uk, w_uv, w_o):
        B, Sq, M = (x.shape[0], x.shape[1], x.shape[2])
        Sk = c_kv.shape[1]
        H, D = (w_q.shape[1], w_q.shape[2])
        q = jnp.einsum('bqm,mhd->bhqd', x, w_q)
        k = jnp.einsum('bkc,chd->bhkd', c_kv, w_uk)
        v = jnp.einsum('bkc,chd->bhkd', c_kv, w_uv)
        scores = jnp.einsum('bhqd,bhkd->bhqk', q, k) * D ** (-0.5)
        off = Sk - Sq
        qi = jnp.arange(Sq)[:, None]
        kj = jnp.arange(Sk)[None, :]
        cmask = kj <= qi + off
        scores = jnp.where(cmask[None, None], scores, -1000000000.0)
        p = _softmax(scores, axis=-1)
        ctx = jnp.einsum('bhqk,bhkd->bhqd', p, v)
        return jnp.einsum('bhqd,hdm->bqm', ctx, w_o)

    def _B_ref(x, w1, w2):
        h = jnp.einsum('bsd,df->bsf', x, w1)
        zero = jnp.zeros_like(h)
        h = jnp.maximum(h, zero)
        return jnp.einsum('bsf,fd->bsd', h, w2)
    x = A_x
    mod = (_silu(c) @ w_mod).reshape(c.shape[0], 6, 1, -1)
    sa, ca, ga, sb, cb, gb = (mod[:, 0].copy(), mod[:, 1].copy(), mod[:, 2].copy(), mod[:, 3].copy(), mod[:, 4].copy(), mod[:, 5].copy())
    h = _layernorm(x, axis=-1) * (1 + ca) + sa
    x = x + ga * _A_ref(h, A_c_kv, A_w_q, A_w_uk, A_w_uv, A_w_o)
    h = _layernorm(x, axis=-1) * (1 + cb) + sb
    x = x + gb * _B_ref(h, B_w1, B_w2)
    return x
```

```python
import functools

import jax
import jax.experimental.pallas as pl
import jax.experimental.pallas.tpu as pltpu
import jax.numpy as jnp
from jax import lax

_F32 = jnp.float32
_BF16 = jnp.bfloat16
_LANES = 128
_KV_CHUNK = 1024
_W2_TAIL = 256
_NT = (((1,), (1,)), ((), ()))


def _dot(a, b):
    return jnp.dot(a, b, preferred_element_type=_F32)


def _dot_nt(a, b):
    return lax.dot_general(a, b, _NT, preferred_element_type=_F32)


def _layernorm(x):
    xc = x - jnp.mean(x, axis=-1, keepdims=True)
    var = jnp.mean(xc * xc, axis=-1, keepdims=True)
    return xc * lax.rsqrt(var + 1e-5)


def _kernel(
    x_hbm, ckv_hbm, wq_hbm, wuk_hbm, wuv_hbm, wo_hbm, w1_hbm, w2_hbm, c_hbm, wmod_hbm,
    out_ref,
    x_v, c_v, wmod_v, wq_v, wuk_v, ckv_v, wuv_v, wo_v, w1_v, w2_v,
    pair_s, q_s, qabs_s, s_s, ctx_s, o_s, sems, kv_sems,
    *, B, H, D, Sk, M, Dc, Dff,
):
    P = H // 2
    w2_head = Dff - _W2_TAIL

    def copy(i, src, dst):
        return pltpu.make_async_copy(src, dst, sems.at[i])

    def kv_copy(b):
        return pltpu.make_async_copy(ckv_hbm.at[b], ckv_v.at[b], kv_sems.at[b])

    cp_wmod = copy(0, wmod_hbm, wmod_v)
    cp_c = copy(1, c_hbm, c_v)
    cp_x = copy(2, x_hbm, x_v)
    cp_wq = copy(3, wq_hbm, wq_v)
    cp_wuk = copy(4, wuk_hbm, wuk_v)
    cp_wuv = copy(5, wuv_hbm, wuv_v)
    cp_wo = copy(6, wo_hbm, wo_v)
    cp_w1 = copy(7, w1_hbm, w1_v)
    cp_w2a = copy(8, w2_hbm.at[pl.ds(0, w2_head)], w2_v.at[pl.ds(0, w2_head)])
    cp_w2b = copy(9, w2_hbm.at[pl.ds(w2_head, _W2_TAIL)], w2_v.at[pl.ds(w2_head, _W2_TAIL)])

    for cp in (cp_wmod, cp_c, cp_x, cp_wq, cp_wuk):
        cp.start()
    for b in range(B):
        kv_copy(b).start()
    for cp in (cp_wuv, cp_wo, cp_w1, cp_w2a, cp_w2b):
        cp.start()

    def stage_pairs(w_v, rows):
        step = 32

        def body(i, carry):
            src = pl.multiple_of(i * (step * H), step * H)
            dst = pl.multiple_of(i * (step * P), step * P)
            pair_s[pl.ds(dst, step * P), :] = pltpu.bitcast(
                w_v[pl.ds(src, step * H), :], jnp.int32)
            return carry

        lax.fori_loop(0, rows // step, body, 0)

    def head_pair(j, rows):
        u = pair_s[pl.ds(j, rows, stride=P), :]
        lo = pltpu.bitcast(u << 16, _F32).astype(_BF16)
        hi = pltpu.bitcast(u & -65536, _F32).astype(_BF16)
        return lo, hi

    cp_c.wait()
    cp_x.wait()
    cp_wmod.wait()
    cf = c_v[...].astype(_F32)
    mod = _dot((cf * jax.nn.sigmoid(cf)).astype(_BF16), wmod_v[...])
    sa, ca, ga, sb, cb, gb = (mod[:, i * M:(i + 1) * M] for i in range(6))
    x = x_v[...].astype(_F32).reshape(B, M)
    h = (_layernorm(x) * (1.0 + ca) + sa).astype(_BF16)

    cp_wq.wait()
    stage_pairs(wq_v, M)

    def q_body(j, carry):
        for e, w in enumerate(head_pair(j, M)):
            q_s[pl.ds(pl.multiple_of((2 * j + e) * B, B), B), :] = _dot(h, w)
        return carry

    lax.fori_loop(0, P, q_body, 0)

    cp_wuk.wait()
    stage_pairs(wuk_v, Dc)

    def qabs_body(j, carry):
        for e, w in enumerate(head_pair(j, Dc)):
            rows = pl.ds(pl.multiple_of((2 * j + e) * B, B), B)
            qa = _dot_nt(q_s[rows, :].astype(_BF16), w) * (D ** -0.5)
            for t in range(Dc // _LANES):
                qabs_s[t, rows, :] = qa[:, t * _LANES:(t + 1) * _LANES]
        return carry

    lax.fori_loop(0, P, qabs_body, 0)

    n_chunks = Sk // _KV_CHUNK

    def batch_body(b, carry):
        qb = jnp.concatenate(
            [qabs_s[t, pl.ds(b, H, stride=B), :] for t in range(Dc // _LANES)], axis=1
        ).astype(_BF16)
        kv_copy(b).wait()

        def keys(i):
            return ckv_v[b, pl.ds(pl.multiple_of(i * _KV_CHUNK, _KV_CHUNK), _KV_CHUNK), :]

        def fold(v, op):
            r = v[:, :_LANES]
            for t in range(1, _KV_CHUNK // _LANES):
                r = op(r, v[:, t * _LANES:(t + 1) * _LANES])
            return r

        def score_body(i, m):
            s = _dot_nt(qb, keys(i))
            s_s[i] = s
            return jnp.maximum(m, fold(s, jnp.maximum))

        m = lax.fori_loop(0, n_chunks, score_body, jnp.full((H, _LANES), -jnp.inf, _F32))
        m = jnp.max(m, axis=-1, keepdims=True)

        def value_body(i, state):
            l, acc = state
            p = jnp.exp(s_s[i] - m)
            return l + fold(p, jnp.add), acc + _dot(p.astype(_BF16), keys(i))

        l, acc = lax.fori_loop(
            0, n_chunks, value_body,
            (jnp.zeros((H, _LANES), _F32), jnp.zeros((H, Dc), _F32)))
        ctx = acc / jnp.sum(l, axis=-1, keepdims=True)
        for t in range(Dc // _LANES):
            ctx_s[t, pl.ds(pl.multiple_of(b * H, H), H), :] = ctx[:, t * _LANES:(t + 1) * _LANES]
        return carry

    lax.fori_loop(0, B, batch_body, 0)

    cp_wuv.wait()
    stage_pairs(wuv_v, Dc)

    def o_body(j, carry):
        for e, w in enumerate(head_pair(j, Dc)):
            ch = jnp.concatenate(
                [ctx_s[t, pl.ds(2 * j + e, B, stride=H), :] for t in range(Dc // _LANES)],
                axis=1)
            o_s[2 * j + e] = _dot(ch.astype(_BF16), w)
        return carry

    lax.fori_loop(0, P, o_body, 0)

    cp_wo.wait()
    heads_per_step = 8

    def proj_body(i, acc):
        o = jnp.concatenate(
            [o_s[i * heads_per_step + k] for k in range(heads_per_step)], axis=1)
        rows = pl.ds(pl.multiple_of(i * (heads_per_step * D), heads_per_step * D),
                     heads_per_step * D)
        return acc + _dot(o.astype(_BF16), wo_v[rows, :])

    attn = lax.fori_loop(0, H // heads_per_step, proj_body, jnp.zeros((B, M), _F32))
    x = x + ga * attn
    h2 = (_layernorm(x) * (1.0 + cb) + sb).astype(_BF16)

    cp_w1.wait()
    f = jnp.maximum(_dot(h2, w1_v[...]), 0.0).astype(_BF16)
    cp_w2a.wait()
    y = _dot(f[:, :w2_head], w2_v[pl.ds(0, w2_head), :])
    cp_w2b.wait()
    y = y + _dot(f[:, w2_head:], w2_v[pl.ds(w2_head, _W2_TAIL), :])
    out_ref[...] = (x + gb * y).reshape(B, 1, M).astype(out_ref.dtype)


@jax.jit
def pallas_adaLN_cond__compressed_kv_cla__dense_activation_relu__decode_kernel(
    A_x: jax.Array,
    A_c_kv: jax.Array,
    A_w_q: jax.Array,
    A_w_uk: jax.Array,
    A_w_uv: jax.Array,
    A_w_o: jax.Array,
    B_x: jax.Array,
    B_w1: jax.Array,
    B_w2: jax.Array,
    c: jax.Array,
    w_mod: jax.Array,
):
    del B_x
    B, Sq, M = A_x.shape
    _, Sk, Dc = A_c_kv.shape
    _, H, D = A_w_q.shape
    Dff = B_w1.shape[1]
    assert Sq == 1 and D == _LANES and B == 8 and H % 16 == 0
    assert Sk % _KV_CHUNK == 0

    operands = (
        A_x,
        A_c_kv,
        A_w_q.reshape(M * H, D),
        A_w_uk.reshape(Dc * H, D),
        A_w_uv.reshape(Dc * H, D),
        A_w_o.reshape(H * D, M),
        B_w1,
        B_w2,
        c,
        w_mod,
    )
    vmem = lambda a: pltpu.VMEM(a.shape, a.dtype)
    x, ckv, wq, wuk, wuv, wo, w1, w2, c, wmod = operands
    scratch_shapes = [
        vmem(x), vmem(c), vmem(wmod), vmem(wq), vmem(wuk), vmem(ckv), vmem(wuv),
        vmem(wo), vmem(w1), vmem(w2),
        pltpu.VMEM(((max(M, Dc) + 1) * (H // 2), D), jnp.int32),
        pltpu.VMEM((H * B, D), _F32),
        pltpu.VMEM((Dc // _LANES, (H + 1) * B, _LANES), _F32),
        pltpu.VMEM((Sk // _KV_CHUNK, H, _KV_CHUNK), _F32),
        pltpu.VMEM((Dc // _LANES, (B + 1) * H, _LANES), _F32),
        pltpu.VMEM((H, B, D), _F32),
        pltpu.SemaphoreType.DMA((10,)),
        pltpu.SemaphoreType.DMA((B,)),
    ]
    return pl.pallas_call(
        functools.partial(_kernel, B=B, H=H, D=D, Sk=Sk, M=M, Dc=Dc, Dff=Dff),
        in_specs=[pl.BlockSpec(memory_space=pl.ANY)] * len(operands),
        out_shape=jax.ShapeDtypeStruct(A_x.shape, A_x.dtype),
        scratch_shapes=scratch_shapes,
        compiler_params=pltpu.CompilerParams(vmem_limit_bytes=100 * 2**20),
    )(*operands)
```

```python
import functools

import jax
import jax.experimental.pallas as pl
import jax.experimental.pallas.tpu as pltpu
import jax.numpy as jnp
from jax import lax

_F32 = jnp.float32
_BF16 = jnp.bfloat16
_LANES = 128
_KV_CHUNK = 1024
_AHEAD = 3
_PRIO = 1
_W2_SPLIT = (None, 768, 256, 128)
_NT = (((1,), (1,)), ((), ()))


def _dot(a, b):
    return jnp.dot(a, b, preferred_element_type=_F32)


def _dot_nt(a, b):
    return lax.dot_general(a, b, _NT, preferred_element_type=_F32)


def _layernorm(x):
    xc = x - jnp.mean(x, axis=-1, keepdims=True)
    var = jnp.mean(xc * xc, axis=-1, keepdims=True)
    return xc * lax.rsqrt(var + 1e-5)


def _kernel(*refs, **dims):
    *refs, out_v = refs
    out_hbm = refs[10]

    def scoped(sems, kv_sems):
        out_v[...] = _block(*refs[:10], *refs[11:], sems, kv_sems, **dims).astype(out_v.dtype)
        write_back = pltpu.make_async_copy(out_v, out_hbm, sems.at[0])
        write_back.start()
        write_back.wait()

    pl.run_scoped(
        scoped,
        pltpu.SemaphoreType.DMA((6 + len(_W2_SPLIT),)),
        pltpu.SemaphoreType.DMA((dims["B"],)),
    )


def _block(
    x_hbm, ckv_hbm, wq_hbm, wuk_hbm, wuv_hbm, wo_hbm, w1_hbm, w2_hbm, c_hbm, wmod_hbm,
    x_v, c_v, wmod_v, wq_v, wuk_v, ckv_v, wuv_v, wo_v, w1_v, w2_v,
    pair_s, q_s, qabs_s, s_s, ctx_s, o_s, sems, kv_sems,
    *, B, H, D, Sk, M, Dc, Dff,
):
    P = H // 2

    def copy(i, src, dst):
        return pltpu.make_async_copy(src, dst, sems.at[i])

    def kv_copy(b):
        return pltpu.make_async_copy(ckv_hbm.at[b], ckv_v.at[b], kv_sems.at[b])

    mod_copies = [copy(0, wmod_hbm, wmod_v), copy(0, c_hbm, c_v), copy(0, x_hbm, x_v)]
    cp_wq = copy(1, wq_hbm, wq_v)
    cp_wuk = copy(2, wuk_hbm, wuk_v)
    cp_wuv = copy(3, wuv_hbm, wuv_v)
    cp_wo = copy(4, wo_hbm, wo_v)
    cp_w1 = copy(5, w1_hbm, w1_v)
    w2_rows, start = [], 0
    for n in (Dff - sum(_W2_SPLIT[1:]),) + _W2_SPLIT[1:]:
        w2_rows.append(slice(start, start + n))
        start += n
    w2_copies = [copy(6 + i, w2_hbm.at[r], w2_v.at[r]) for i, r in enumerate(w2_rows)]

    for cp in mod_copies + [cp_wq, cp_wuk]:
        cp.start(priority=_PRIO)

    def stage_pairs(w_v, rows):
        step = 32

        def body(i, carry):
            src = pl.multiple_of(i * (step * H), step * H)
            dst = pl.multiple_of(i * (step * P), step * P)
            pair_s[pl.ds(dst, step * P), :] = pltpu.bitcast(
                w_v[pl.ds(src, step * H), :], jnp.int32)
            return carry

        lax.fori_loop(0, rows // step, body, 0)

    def head_pair(j, rows):
        u = pair_s[pl.ds(j, rows, stride=P), :]
        lo = pltpu.bitcast(u << 16, _F32).astype(_BF16)
        hi = pltpu.bitcast(u & -65536, _F32).astype(_BF16)
        return lo, hi

    for cp in mod_copies:
        cp.wait()
    kv_copy(0).start(priority=_PRIO)
    cf = c_v[...].astype(_F32)
    mod = _dot((cf * jax.nn.sigmoid(cf)).astype(_BF16), wmod_v[...])
    sa, ca, ga, sb, cb, gb = (mod[:, i * M:(i + 1) * M] for i in range(6))
    x = x_v[...].astype(_F32)
    h = (_layernorm(x) * (1.0 + ca) + sa).astype(_BF16)

    cp_wq.wait()
    kv_copy(1).start(priority=_PRIO)
    stage_pairs(wq_v, M)

    def q_body(j, carry):
        for e, w in enumerate(head_pair(j, M)):
            q_s[pl.ds(pl.multiple_of((2 * j + e) * B, B), B), :] = _dot(h, w)
        return carry

    lax.fori_loop(0, P, q_body, 0)

    cp_wuk.wait()
    kv_copy(2).start(priority=_PRIO)
    stage_pairs(wuk_v, Dc)

    def qabs_body(j, carry):
        for e, w in enumerate(head_pair(j, Dc)):
            rows = pl.ds(pl.multiple_of((2 * j + e) * B, B), B)
            qa = _dot_nt(q_s[rows, :].astype(_BF16), w) * (D ** -0.5)
            for t in range(Dc // _LANES):
                qabs_s[t, rows, :] = qa[:, t * _LANES:(t + 1) * _LANES]
        return carry

    lax.fori_loop(0, P, qabs_body, 0)

    n_chunks = Sk // _KV_CHUNK

    def batch_body(b, carry):
        qb = jnp.concatenate(
            [qabs_s[t, pl.ds(b, H, stride=B), :] for t in range(Dc // _LANES)], axis=1
        ).astype(_BF16)
        kv_copy(b).wait()

        @pl.when(b + _AHEAD < B)
        def _():
            kv_copy(b + _AHEAD).start(priority=_PRIO)

        for k, cp in enumerate((cp_wuv, cp_wo, cp_w1)):
            pl.when(b + _AHEAD == B + k)(functools.partial(cp.start, priority=_PRIO))

        def keys(i):
            return ckv_v[b, pl.ds(pl.multiple_of(i * _KV_CHUNK, _KV_CHUNK), _KV_CHUNK), :]

        def fold(v, op):
            r = v[:, :_LANES]
            for t in range(1, _KV_CHUNK // _LANES):
                r = op(r, v[:, t * _LANES:(t + 1) * _LANES])
            return r

        def score_body(i, m):
            s = _dot_nt(qb, keys(i))
            s_s[i] = s
            return jnp.maximum(m, fold(s, jnp.maximum))

        m = lax.fori_loop(0, n_chunks, score_body, jnp.full((H, _LANES), -jnp.inf, _F32))
        m = jnp.max(m, axis=-1, keepdims=True)

        def value_body(i, state):
            l, acc = state
            p = jnp.exp(s_s[i] - m)
            return l + fold(p, jnp.add), acc + _dot(p.astype(_BF16), keys(i))

        l, acc = lax.fori_loop(
            0, n_chunks, value_body,
            (jnp.zeros((H, _LANES), _F32), jnp.zeros((H, Dc), _F32)))
        ctx = acc / jnp.sum(l, axis=-1, keepdims=True)
        for t in range(Dc // _LANES):
            ctx_s[t, pl.ds(pl.multiple_of(b * H, H), H), :] = ctx[:, t * _LANES:(t + 1) * _LANES]
        return carry

    lax.fori_loop(0, B, batch_body, 0)

    cp_wuv.wait()
    for cp in w2_copies:
        cp.start(priority=_PRIO)
    stage_pairs(wuv_v, Dc)

    def o_body(j, carry):
        for e, w in enumerate(head_pair(j, Dc)):
            ch = jnp.concatenate(
                [ctx_s[t, pl.ds(2 * j + e, B, stride=H), :] for t in range(Dc // _LANES)],
                axis=1)
            o_s[2 * j + e] = _dot(ch.astype(_BF16), w)
        return carry

    lax.fori_loop(0, P, o_body, 0)

    cp_wo.wait()
    heads_per_step = 8

    def proj_body(i, acc):
        o = jnp.concatenate(
            [o_s[i * heads_per_step + k] for k in range(heads_per_step)], axis=1)
        rows = pl.ds(pl.multiple_of(i * (heads_per_step * D), heads_per_step * D),
                     heads_per_step * D)
        return acc + _dot(o.astype(_BF16), wo_v[rows, :])

    attn = lax.fori_loop(0, H // heads_per_step, proj_body, jnp.zeros((B, M), _F32))
    x = x + ga * attn
    h2 = (_layernorm(x) * (1.0 + cb) + sb).astype(_BF16)

    cp_w1.wait()
    f = jnp.maximum(_dot(h2, w1_v[...]), 0.0).astype(_BF16)
    for cp, r in zip(w2_copies, w2_rows):
        cp.wait()
        x = x + gb * _dot(f[:, r], w2_v[r, :])
    return x


@jax.jit
def pallas_adaLN_cond__compressed_kv_cla__dense_activation_relu__decode_kernel(
    A_x: jax.Array,
    A_c_kv: jax.Array,
    A_w_q: jax.Array,
    A_w_uk: jax.Array,
    A_w_uv: jax.Array,
    A_w_o: jax.Array,
    B_x: jax.Array,
    B_w1: jax.Array,
    B_w2: jax.Array,
    c: jax.Array,
    w_mod: jax.Array,
):
    del B_x
    B, Sq, M = A_x.shape
    _, Sk, Dc = A_c_kv.shape
    _, H, D = A_w_q.shape
    Dff = B_w1.shape[1]
    assert Sq == 1 and D == _LANES and B == 8 and H % 16 == 0
    assert Sk % _KV_CHUNK == 0

    operands = (
        A_x.reshape(B, M),
        A_c_kv,
        A_w_q.reshape(M * H, D),
        A_w_uk.reshape(Dc * H, D),
        A_w_uv.reshape(Dc * H, D),
        A_w_o.reshape(H * D, M),
        B_w1,
        B_w2,
        c,
        w_mod,
    )
    vmem = lambda a: pltpu.VMEM(a.shape, a.dtype)
    x, ckv, wq, wuk, wuv, wo, w1, w2, c, wmod = operands
    scratch_shapes = [
        vmem(x), vmem(c), vmem(wmod), vmem(wq), vmem(wuk), vmem(ckv), vmem(wuv),
        vmem(wo), vmem(w1), vmem(w2),
        pltpu.VMEM(((max(M, Dc) + 1) * (H // 2), D), jnp.int32),
        pltpu.VMEM((H * B, D), _F32),
        pltpu.VMEM((Dc // _LANES, (H + 1) * B, _LANES), _F32),
        pltpu.VMEM((Sk // _KV_CHUNK, H, _KV_CHUNK), _F32),
        pltpu.VMEM((Dc // _LANES, (B + 1) * H, _LANES), _F32),
        pltpu.VMEM((H, B, D), _F32),
        vmem(x),
    ]
    out = pl.pallas_call(
        functools.partial(_kernel, B=B, H=H, D=D, Sk=Sk, M=M, Dc=Dc, Dff=Dff),
        in_specs=[pl.BlockSpec(memory_space=pl.ANY)] * len(operands),
        out_specs=pl.BlockSpec(memory_space=pl.ANY),
        out_shape=jax.ShapeDtypeStruct((B, M), A_x.dtype),
        scratch_shapes=scratch_shapes,
        compiler_params=pltpu.CompilerParams(vmem_limit_bytes=100 * 2**20),
    )(*operands)
    return out.reshape(B, Sq, M)
```

```python
import functools

import jax
import jax.experimental.pallas as pl
import jax.experimental.pallas.tpu as pltpu
import jax.numpy as jnp
from jax import lax

_F32 = jnp.float32
_BF16 = jnp.bfloat16
_LANES = 128
_KV_CHUNK = 1024
_W2_TAIL = (768, 256, 128)


def _dot(a, b):
    return jnp.dot(a, b, preferred_element_type=_F32)


def _dot_nt(a, b):
    return lax.dot_general(a, b, (((1,), (1,)), ((), ())), preferred_element_type=_F32)


def _layernorm(x):
    xc = x - jnp.mean(x, axis=-1, keepdims=True)
    var = jnp.mean(xc * xc, axis=-1, keepdims=True)
    return xc * lax.rsqrt(var + 1e-5)


def _rows(i, n):
    return pl.ds(pl.multiple_of(i * n, n), n)


def _lane_tiles(v):
    return [v[:, t:t + _LANES] for t in range(0, v.shape[1], _LANES)]


def _block(
    x_hbm, ckv_hbm, wq_hbm, wuk_hbm, wuv_hbm, wo_hbm, w1_hbm, w2_hbm, c_hbm, wmod_hbm,
    out_ref,
    x_v, ckv_v, wq_v, wuk_v, wuv_v, wo_v, w1_v, w2_v, c_v, wmod_v,
    pair_s, q_s, qabs_s, s_s, ctx_s, o_s,
    sems, kv_sems,
):
    B, Sk, Dc = ckv_v.shape
    H, _, D = o_s.shape
    M, Dff = w1_v.shape
    P = H // 2

    def copy(i, src, dst):
        return pltpu.make_async_copy(src, dst, sems.at[i])

    def kv_copy(b):
        return pltpu.make_async_copy(ckv_hbm.at[b], ckv_v.at[b], kv_sems.at[b])

    mod_copies = [copy(0, wmod_hbm, wmod_v), copy(0, c_hbm, c_v), copy(0, x_hbm, x_v)]
    cp_wq = copy(1, wq_hbm, wq_v)
    cp_wuk = copy(2, wuk_hbm, wuk_v)
    cp_wuv = copy(3, wuv_hbm, wuv_v)
    cp_wo = copy(4, wo_hbm, wo_v)
    cp_w1 = copy(5, w1_hbm, w1_v)
    w2_rows, start = [], 0
    for n in (Dff - sum(_W2_TAIL),) + _W2_TAIL:
        w2_rows.append(slice(start, start + n))
        start += n
    w2_copies = [copy(6 + i, w2_hbm.at[r], w2_v.at[r]) for i, r in enumerate(w2_rows)]

    for cp in mod_copies + [cp_wq, cp_wuk]:
        cp.start()

    def stage_pairs(w_v):
        step = 32

        def body(i, carry):
            pair_s[_rows(i, step * P), :] = pltpu.bitcast(
                w_v[_rows(i, step * H), :], jnp.int32)
            return carry

        lax.fori_loop(0, w_v.shape[0] // (step * H), body, 0)

    def head_pair(j, rows):
        u = pair_s[pl.ds(j, rows, stride=P), :]
        lo = pltpu.bitcast(u << 16, _F32).astype(_BF16)
        hi = pltpu.bitcast(u & -65536, _F32).astype(_BF16)
        return lo, hi

    for cp in mod_copies:
        cp.wait()
    kv_copy(0).start()
    cf = c_v[...].astype(_F32)
    mod = _dot((cf * jax.nn.sigmoid(cf)).astype(_BF16), wmod_v[...])
    sa, ca, ga, sb, cb, gb = (mod[:, i * M:(i + 1) * M] for i in range(6))
    x = x_v[...].astype(_F32)
    h = (_layernorm(x) * (1.0 + ca) + sa).astype(_BF16)

    cp_wq.wait()
    kv_copy(1).start()
    stage_pairs(wq_v)

    def q_body(j, carry):
        for e, w in enumerate(head_pair(j, M)):
            q_s[2 * j + e] = _dot(h, w)
        return carry

    lax.fori_loop(0, P, q_body, 0)

    cp_wuk.wait()
    kv_copy(2).start()
    stage_pairs(wuk_v)

    def qabs_body(j, carry):
        for e, w in enumerate(head_pair(j, Dc)):
            qa = _dot_nt(q_s[2 * j + e].astype(_BF16), w) * (D ** -0.5)
            for t, tile in enumerate(_lane_tiles(qa)):
                qabs_s[t, _rows(2 * j + e, B), :] = tile
        return carry

    lax.fori_loop(0, P, qabs_body, 0)

    n_chunks = Sk // _KV_CHUNK

    def batch_body(b, carry):
        qb = jnp.concatenate(
            [qabs_s[t, pl.ds(b, H, stride=B), :] for t in range(Dc // _LANES)], axis=1
        ).astype(_BF16)
        kv_copy(b).wait()

        @pl.when(b + 3 < B)
        def _():
            kv_copy(b + 3).start()

        for k, cp in enumerate((cp_wuv, cp_wo, cp_w1)):
            pl.when(b + 3 == B + k)(cp.start)

        def score_body(i, m):
            s = _dot_nt(qb, ckv_v[b, _rows(i, _KV_CHUNK), :])
            s_s[i] = s
            return functools.reduce(jnp.maximum, _lane_tiles(s), m)

        m = lax.fori_loop(0, n_chunks, score_body, jnp.full((H, _LANES), -jnp.inf, _F32))
        m = jnp.max(m, axis=-1, keepdims=True)

        def value_body(i, state):
            l, acc = state
            p = jnp.exp(s_s[i] - m)
            l = functools.reduce(jnp.add, _lane_tiles(p), l)
            return l, acc + _dot(p.astype(_BF16), ckv_v[b, _rows(i, _KV_CHUNK), :])

        l, acc = lax.fori_loop(
            0, n_chunks, value_body,
            (jnp.zeros((H, _LANES), _F32), jnp.zeros((H, Dc), _F32)))
        ctx = acc / jnp.sum(l, axis=-1, keepdims=True)
        for t, tile in enumerate(_lane_tiles(ctx)):
            ctx_s[t, _rows(b, H), :] = tile
        return carry

    lax.fori_loop(0, B, batch_body, 0)

    cp_wuv.wait()
    for cp in w2_copies:
        cp.start()
    stage_pairs(wuv_v)

    def o_body(j, carry):
        for e, w in enumerate(head_pair(j, Dc)):
            ch = jnp.concatenate(
                [ctx_s[t, pl.ds(2 * j + e, B, stride=H), :] for t in range(Dc // _LANES)],
                axis=1)
            o_s[2 * j + e] = _dot(ch.astype(_BF16), w)
        return carry

    lax.fori_loop(0, P, o_body, 0)

    cp_wo.wait()
    group = 8

    def proj_body(i, acc):
        o = jnp.concatenate([o_s[i * group + k] for k in range(group)], axis=1)
        return acc + _dot(o.astype(_BF16), wo_v[_rows(i, group * D), :])

    attn = lax.fori_loop(0, H // group, proj_body, jnp.zeros((B, M), _F32))
    x = x + ga * attn
    h2 = (_layernorm(x) * (1.0 + cb) + sb).astype(_BF16)

    cp_w1.wait()
    f = jnp.maximum(_dot(h2, w1_v[...]), 0.0).astype(_BF16)
    for cp, r in zip(w2_copies, w2_rows):
        cp.wait()
        x = x + gb * _dot(f[:, r], w2_v[r, :])
    out_ref[...] = x.astype(out_ref.dtype)


def _kernel(*refs):
    pl.run_scoped(
        functools.partial(_block, *refs),
        pltpu.SemaphoreType.DMA((7 + len(_W2_TAIL),)),
        pltpu.SemaphoreType.DMA((refs[1].shape[0],)),
    )


@jax.jit
def pallas_adaLN_cond__compressed_kv_cla__dense_activation_relu__decode_kernel(
    A_x: jax.Array,
    A_c_kv: jax.Array,
    A_w_q: jax.Array,
    A_w_uk: jax.Array,
    A_w_uv: jax.Array,
    A_w_o: jax.Array,
    B_x: jax.Array,
    B_w1: jax.Array,
    B_w2: jax.Array,
    c: jax.Array,
    w_mod: jax.Array,
):
    del B_x
    B, Sq, M = A_x.shape
    _, Sk, Dc = A_c_kv.shape
    _, H, D = A_w_q.shape
    assert Sq == 1 and B == 8 and D == _LANES and H % 16 == 0 and Sk % _KV_CHUNK == 0

    operands = (
        A_x.reshape(B, M),
        A_c_kv,
        A_w_q.reshape(M * H, D),
        A_w_uk.reshape(Dc * H, D),
        A_w_uv.reshape(Dc * H, D),
        A_w_o.reshape(H * D, M),
        B_w1,
        B_w2,
        c,
        w_mod,
    )
    assert all(a.dtype == _BF16 for a in operands)
    scratch_shapes = [pltpu.VMEM(a.shape, a.dtype) for a in operands] + [
        pltpu.VMEM(((max(M, Dc) + 1) * (H // 2), D), jnp.int32),
        pltpu.VMEM((H, B, D), _F32),
        pltpu.VMEM((Dc // _LANES, (H + 1) * B, _LANES), _F32),
        pltpu.VMEM((Sk // _KV_CHUNK, H, _KV_CHUNK), _F32),
        pltpu.VMEM((Dc // _LANES, (B + 1) * H, _LANES), _F32),
        pltpu.VMEM((H, B, D), _F32),
    ]
    out = pl.pallas_call(
        _kernel,
        in_specs=[pl.BlockSpec(memory_space=pl.ANY)] * len(operands),
        out_shape=jax.ShapeDtypeStruct((B, M), A_x.dtype),
        scratch_shapes=scratch_shapes,
        compiler_params=pltpu.CompilerParams(vmem_limit_bytes=80 * 2**20),
    )(*operands)
    return out.reshape(B, Sq, M)
```
